```python
import os as _os
_os.environ.setdefault("JAX_PLATFORMS", "cpu")
import jax
import jax.numpy as jnp

def _softmax(x, axis=-1):
    return jax.nn.softmax(x, axis=axis)
def _gelu(x):
    return jax.nn.gelu(x, approximate=True)
def _silu(x):
    return jax.nn.silu(x)
def _sigmoid(x):
    return jax.nn.sigmoid(x)
def _layernorm(x, axis=-1, eps=1e-5):
    m = jnp.mean(x, axis=axis, keepdims=True)
    v = jnp.var(x, axis=axis, keepdims=True)
    return (x - m) / jnp.sqrt(v + eps)
def _scatter_add(tgt, idx, src, axis=0):
    return tgt.at[idx].add(src)
def _segment_sum(src, seg, n):
    return jax.ops.segment_sum(src, seg, n)
class _Rng:
    def __init__(self, key):
        self._k = key
    def _next(self):
        self._k, sub = jax.random.split(self._k)
        return sub
    def normal(self, shape):
        return jax.random.normal(self._next(), shape, dtype=jnp.bfloat16)
    def randint(self, lo, hi, shape):
        return jax.random.randint(self._next(), shape, lo, hi, dtype=jnp.int32)
    def uniform(self, shape, lo=0.0, hi=1.0):
        return jax.random.uniform(self._next(), shape, jnp.bfloat16, lo, hi)
    def permutation(self, n):
        return jax.random.permutation(self._next(), n)


kernel_name = 'standalone__dense_activation_gelu__prompt'

def setup_inputs():
    _rng = _Rng(jax.random.key(int.from_bytes(__import__("os").urandom(4), "little")))
    _w = (lambda a: (lambda t: t.astype(jnp.bfloat16) if jnp.issubdtype(t.dtype, jnp.floating) else t)(jnp.asarray(a)))
    B, S, D, F = 1, 2048, 640, 1728
    return {
        "x": _w((lambda *s: _rng.normal(s) * 0.05)(B, S, D)),
        "w1": _w((lambda *s: _rng.normal(s) * 0.05)(D, F) * (D ** -0.5)),
        "b1": _w((lambda *s: _rng.normal(s) * 0.05)(F) * 0.01),
        "w2": _w((lambda *s: _rng.normal(s) * 0.05)(F, D) * (F ** -0.5)),
        "b2": _w((lambda *s: _rng.normal(s) * 0.05)(D) * 0.01),
    }

def reference(x, w1, b1, w2, b2):
    h = jnp.einsum("bsd,df->bsf", x, w1) + b1
    h = _gelu(h)
    return jnp.einsum("bsf,fd->bsd", h, w2) + b2
```

```python
import jax
import jax.numpy as jnp
from jax import lax
import jax.experimental.pallas as pl
import jax.experimental.pallas.tpu as pltpu

_SQRT_2_OVER_PI = 0.7978845608028654


def _gelu_tanh(h):
    return 0.5 * h * (1.0 + jnp.tanh(_SQRT_2_OVER_PI * (h + 0.044715 * (h * h * h))))


def _dot_nt(a, b):
    return lax.dot_general(a, b, (((1,), (1,)), ((), ())),
                           preferred_element_type=jnp.float32)


def _dot_nn(a, b):
    return jnp.dot(a, b, preferred_element_type=jnp.float32)


def _plan(S, D, F):
    tm = 512 if (S % 512 == 0 and S >= 1024) else S
    blocks = (tm,) * (S // tm)
    cuts = tuple(c for c in (256, 768) if c < F) if len(blocks) > 1 else ()
    if D % 128 == 0 and D >= 512:
        colsplit = (D - 384, 256, 128)
    else:
        colsplit = (D,)
    return blocks, cuts, colsplit


def _make_kernel(blocks, w1cuts, colsplit):
    nb = len(blocks)
    r0s = [sum(blocks[:i]) for i in range(nb)]
    n_out_copies = nb - 1 + len(colsplit)

    def kernel(x_hbm, w1t_hbm, b1_hbm, w2_hbm, b2_hbm, o_hbm,
               x_v, w1t_v, b1_v, w2_v, b2_v, o_v, g_v,
               sem_x, sem_w1, sem_misc, sem_o):
        _, D = x_hbm.shape
        F = w1t_hbm.shape[0]
        cuts = [0] + list(w1cuts) + [F]
        w1ch = [(cuts[i], cuts[i + 1] - cuts[i]) for i in range(len(cuts) - 1)]
        nch = len(w1ch)

        def x_cp(i):
            sl = pl.ds(r0s[i], blocks[i])
            return pltpu.make_async_copy(x_hbm.at[sl, :], x_v.at[sl, :], sem_x.at[i])

        def w1_cp(c):
            sl = pl.ds(*w1ch[c])
            return pltpu.make_async_copy(w1t_hbm.at[sl, :], w1t_v.at[sl, :], sem_w1.at[c])

        w2_cp = pltpu.make_async_copy(w2_hbm, w2_v, sem_misc.at[0])
        b1_cp = pltpu.make_async_copy(b1_hbm, b1_v, sem_misc.at[1])
        b2_cp = pltpu.make_async_copy(b2_hbm, b2_v, sem_misc.at[2])

        out_cps = []

        def start_out(r0, n, c0, cn):
            cp = pltpu.make_async_copy(
                o_v.at[pl.ds(r0, n), pl.ds(c0, cn)],
                o_hbm.at[pl.ds(r0, n), pl.ds(c0, cn)],
                sem_o.at[len(out_cps)])
            cp.start()
            out_cps.append(cp)

        x_cp(0).start()
        w1_cp(0).start()
        b1_cp.start()
        b2_cp.start()
        x_cp(0).wait()
        b1_cp.wait()
        b2_cp.wait()
        pending = ([w1_cp(c) for c in range(1, nch)] + [w2_cp]
                   + [x_cp(i) for i in range(1, nb)])

        def release(n):
            for _ in range(n):
                if pending:
                    pending.pop(0).start()

        release(1)
        w1_cp(0).wait()
        release(1)

        b1 = b1_v[...].astype(jnp.float32).reshape(1, F)
        b2 = b2_v[...].astype(jnp.float32).reshape(1, D)

        def second_matmul(g, r0, n, split):
            c0 = 0
            for cn in split:
                if cn == D:
                    o = _dot_nn(g, w2_v[...]) + b2
                else:
                    o = _dot_nn(g, w2_v[:, pl.ds(c0, cn)]) + b2[:, c0:c0 + cn]
                o_v[pl.ds(r0, n), pl.ds(c0, cn)] = o.astype(o_v.dtype)
                start_out(r0, n, c0, cn)
                c0 += cn

        xb = x_v[pl.ds(0, blocks[0]), :]
        for c, (a, n) in enumerate(w1ch):
            if c > 0:
                w1_cp(c).wait()
                release(1)
            h = _dot_nt(xb, w1t_v[pl.ds(a, n), :]) + b1[:, a:a + n]
            g_v[:, pl.ds(a, n)] = _gelu_tanh(h).astype(jnp.bfloat16)
        w2_cp.wait()
        release(len(pending))
        if nb > 1:
            x_cp(1).wait()
        second_matmul(g_v[...], 0, blocks[0], colsplit if nb == 1 else (D,))

        for i in range(1, nb):
            if i == 2:
                for j in range(2, nb):
                    x_cp(j).wait()
            h = _dot_nt(x_v[pl.ds(r0s[i], blocks[i]), :], w1t_v[...]) + b1
            g = _gelu_tanh(h).astype(jnp.bfloat16)
            second_matmul(g, r0s[i], blocks[i], colsplit if i == nb - 1 else (D,))

        assert len(out_cps) == n_out_copies
        for cp in out_cps:
            cp.wait()

    return kernel, n_out_copies


@jax.jit
def pallas_standalone__dense_activation_gelu__prompt_kernel(
    x: jax.Array,
    w1: jax.Array,
    b1: jax.Array,
    w2: jax.Array,
    b2: jax.Array,
):
    B, S, D = x.shape
    F = w1.shape[1]
    rows = B * S
    blocks, w1cuts, colsplit = _plan(rows, D, F)
    kernel, n_out_copies = _make_kernel(blocks, w1cuts, colsplit)

    out = pl.pallas_call(
        kernel,
        in_specs=[pl.BlockSpec(memory_space=pl.ANY)] * 5,
        out_specs=pl.BlockSpec(memory_space=pl.ANY),
        out_shape=jax.ShapeDtypeStruct((rows, D), x.dtype),
        scratch_shapes=[
            pltpu.VMEM((rows, D), x.dtype),
            pltpu.VMEM((F, D), w1.dtype),
            pltpu.VMEM((F,), b1.dtype),
            pltpu.VMEM((F, D), w2.dtype),
            pltpu.VMEM((D,), b2.dtype),
            pltpu.VMEM((rows, D), x.dtype),
            pltpu.VMEM((blocks[0], F), jnp.bfloat16),
            pltpu.SemaphoreType.DMA((len(blocks),)),
            pltpu.SemaphoreType.DMA((len(w1cuts) + 1,)),
            pltpu.SemaphoreType.DMA((3,)),
            pltpu.SemaphoreType.DMA((n_out_copies,)),
        ],
        compiler_params=pltpu.CompilerParams(
            vmem_limit_bytes=96 * 1024 * 1024,
            disable_semaphore_checks=True,
        ),
    )(x.reshape(rows, D), w1.T, b1, w2, b2)
    return out.reshape(B, S, D)
```
